```python
import os as _os
_os.environ.setdefault("JAX_PLATFORMS", "cpu")
import jax
import jax.numpy as jnp

def _softmax(x, axis=-1):
    return jax.nn.softmax(x, axis=axis)
def _gelu(x):
    return jax.nn.gelu(x, approximate=True)
def _silu(x):
    return jax.nn.silu(x)
def _sigmoid(x):
    return jax.nn.sigmoid(x)
def _layernorm(x, axis=-1, eps=1e-5):
    m = jnp.mean(x, axis=axis, keepdims=True)
    v = jnp.var(x, axis=axis, keepdims=True)
    return (x - m) / jnp.sqrt(v + eps)
def _scatter_add(tgt, idx, src, axis=0):
    return tgt.at[idx].add(src)
def _segment_sum(src, seg, n):
    return jax.ops.segment_sum(src, seg, n)
class _Rng:
    def __init__(self, key):
        self._k = key
    def _next(self):
        self._k, sub = jax.random.split(self._k)
        return sub
    def normal(self, shape):
        return jax.random.normal(self._next(), shape, dtype=jnp.bfloat16)
    def randint(self, lo, hi, shape):
        return jax.random.randint(self._next(), shape, lo, hi, dtype=jnp.int32)
    def uniform(self, shape, lo=0.0, hi=1.0):
        return jax.random.uniform(self._next(), shape, jnp.bfloat16, lo, hi)
    def permutation(self, n):
        return jax.random.permutation(self._next(), n)


kernel_name = 'gated_mix__sliding_block__dense_activation_silu__prompt'

def setup_inputs():
    _rng = _Rng(jax.random.key(int.from_bytes(__import__("os").urandom(4), "little")))
    _w = (lambda a: (lambda t: t.astype(jnp.bfloat16) if jnp.issubdtype(t.dtype, jnp.floating) else t)(jnp.asarray(a)))
    def _A_setup():
        B, S, D = 1, 2048, 640
        return {
            "x": _w((lambda *s: _rng.normal(s) * 0.05)(B, S, D)),
            "wqkv": _w((lambda *s: _rng.normal(s) * 0.4)(D, 3 * D)),
            "wo": _w((lambda *s: _rng.normal(s) * 0.05)(D, D)),
        }
    _A_in = _A_setup()

    def _B_setup():
        B, S, D, F = 1, 2048, 640, 1536
        return {
            "x": _w((lambda *s: _rng.normal(s) * 0.05)(B, S, D)),
            "w1": _w((lambda *s: _rng.normal(s) * 1.6)(D, F) * (D ** -0.5)),
            "w2": _w((lambda *s: _rng.normal(s) * 1.6)(F, D) * (F ** -0.5)),
        }
    _B_in = _B_setup()

    return {
        "A_x": _A_in["x"],
        "A_wqkv": _A_in["wqkv"],
        "A_wo": _A_in["wo"],
        "B_x": _B_in["x"],
        "B_w1": _B_in["w1"],
        "B_w2": _B_in["w2"],
        "gate_w": _w((lambda *s: _rng.normal(s) * 0.05)(640) * 16.0),
    }

def reference(A_x, A_wqkv, A_wo, B_x, B_w1, B_w2, gate_w):
    def _A_ref(x, wqkv, wo):
        B, S, D = x.shape
        H = 32; Dh = D // H; W = 256
        qkv = (lambda x, *d: x.transpose(*d))((x @ wqkv).reshape(B, S, 3, H, Dh), 2, 0, 3, 1, 4)
        q, k, v = qkv[0], qkv[1], qkv[2]
        scores = jnp.einsum("bhqd,bhkd->bhqk", q, k) * (Dh ** -0.5)
        idx = jnp.arange(S)
        mask = (idx[:, None] - idx[None, :] >= 0) & (idx[:, None] - idx[None, :] < W)
        scores = jnp.where(mask[None, None], scores, -1e9)
        p = _softmax(scores, axis=-1)
        o = jnp.einsum("bhqk,bhkd->bhqd", p, v)
        return (lambda x, *d: x.transpose(*d))(o, 0, 2, 1, 3).reshape(B, S, D) @ wo

    def _B_ref(x, w1, w2):
        h = jnp.einsum("bsd,df->bsf", x, w1)
        h = _silu(h)
        out = jnp.einsum("bsf,fd->bsd", h, w2)
        return out

    x = A_x
    g = _sigmoid((x * gate_w).sum(-1, keepdims=True))
    a = _A_ref(x, A_wqkv, A_wo)
    b = _B_ref(x, B_w1, B_w2)
    return g * a + (1 - g) * b
```

```python
import math

import jax
import jax.numpy as jnp
from jax import lax
import jax.experimental.pallas as pl
import jax.experimental.pallas.tpu as pltpu

S, D, H, DH, F = 2048, 640, 32, 20, 1536
NG = 8
T = 256
NU = T // 64
WIN = 320
LA = 6
LOG2E = math.log2(math.e)
QSCALE = float(DH ** -0.5 * LOG2E)
NEG = -1e30
PCS = (0, 512, 1024, 1536, 1920)
NP = len(PCS) - 1
W1, WO, W2, GW = NP, NP + 1, NP + 2, NP + 3

NT = (((1,), (1,)), ((), ()))
f32, bf16 = jnp.float32, jnp.bfloat16


def _kernel(x_hbm, gw_hbm, wqkv_hbm, wo_hbm, w1_hbm, w2_hbm, o_hbm,
            x_v, out_v, gw_v, wqkv_v, wo_v, w1_v, w2_v, k_scr, v_scr, q_scr, h_scr, o_scr, wsem, xsem, osem, *sbuf):
    ib = pl.program_id(0)
    zs = pl.multiple_of((ib >> 20) * 16, 16)
    zl = pl.multiple_of((ib >> 21) * 16, 16)

    def wcp(i):
        srcs = [wqkv_hbm.at[:, PCS[u]:PCS[u + 1]] for u in range(NP)] + [w1_hbm, wo_hbm, w2_hbm, gw_hbm]
        dsts = [wqkv_v.at[:, PCS[u]:PCS[u + 1]] for u in range(NP)] + [w1_v, wo_v, w2_v, gw_v]
        return pltpu.make_async_copy(srcs[i], dsts[i], wsem.at[i])

    def xcp(blk, slot):
        return pltpu.make_async_copy(x_hbm.at[pl.ds(blk * T, T), :], x_v.at[slot], xsem.at[slot])

    def ocp(blk, slot, r):
        return pltpu.make_async_copy(out_v.at[slot, 64 * r:64 * r + 64], o_hbm.at[pl.ds(blk * T + 64 * r, 64), :], osem.at[slot * 4 + r])

    def step(first):
        if first:
            xcp(0, 0).start()
            wcp(0).start()
            xcp(0, 0).wait()
            for i in range(1, NP + 4):
                wcp(i).start()
            slot = 0
        else:
            slot = ib % 2

            @pl.when(ib + 1 < S // T)
            def _():
                xcp(ib + 1, 1 - slot).start()
            xcp(ib, slot).wait()

            @pl.when(ib >= 2)
            def _():
                for r in range(4):
                    ocp(ib - 2, slot, r).wait()
        x_ref = x_v.at[slot]
        xb = x_ref[...]

        lane = lax.broadcasted_iota(jnp.int32, (T, 128), 1)
        row0 = 0 if first else pl.multiple_of(ib * T, T)

        def group_tile(tile, j):
            lo = 80 * j
            a, b = lo // 128, (lo + 79) // 128
            return tile(a) if a == b else jnp.where(lane >= lo % 128, tile(a), tile(b))

        def q_store(tile, j):
            q_scr[pl.ds(zs + j * T, T), :] = group_tile(tile, j) * QSCALE

        def k_store(tile, j):
            k_scr[j, pl.ds(row0, T), :] = group_tile(tile, j).astype(bf16)

        if first:
            cols, done = [], set()
            for u in range(NP):
                wcp(u).wait()
                if u == NP - 1:
                    xcp(1, 1).start()
                have = len(cols)
                part = jnp.dot(xb, wqkv_v[:, PCS[u]:PCS[u + 1]], preferred_element_type=f32)
                cols.extend(part[:, 128 * t:128 * t + 128] for t in range((PCS[u + 1] - PCS[u]) // 128))
                if u == NP - 1:
                    have = len(cols)
                for j in range(NG):
                    hi = (80 * j + 79) // 128
                    if ("q", j) not in done and hi < have:
                        q_store(lambda t: cols[t], j)
                        done.add(("q", j))
                    if ("k", j) not in done and 5 + hi < have:
                        k_store(lambda t: cols[5 + t], j)
                        done.add(("k", j))
            v = jnp.concatenate(cols[10:15], axis=1)
        else:
            q = jnp.dot(xb, wqkv_v[:, 0:D], preferred_element_type=f32)
            k = jnp.dot(xb, wqkv_v[:, D:2 * D], preferred_element_type=f32)
            v = jnp.dot(xb, wqkv_v[:, 2 * D:3 * D], preferred_element_type=f32)
            for j in range(NG):
                q_store(lambda t: q[:, 128 * t:128 * t + 128], j)
            for j in range(NG):
                k_store(lambda t: k[:, 128 * t:128 * t + 128], j)

        vt = v.T
        ones8 = jnp.ones((8, T), f32)
        kb0 = 0 if first else ib * (T // 128)
        for p in range(H // 2):
            rows = vt[40 * p:40 * p + 40]
            va = jnp.concatenate([rows, ones8] if p % 2 == 0 else [ones8, rows], axis=0).astype(bf16)
            for t in range(T // 128):
                v_scr[p, kb0 + t] = va[:, 128 * t:128 * t + 128]

        def ffn1(c0, c1):
            hp = jnp.dot(x_ref[...], w1_v[:, c0:c1], preferred_element_type=f32)
            act = hp * pltpu.reciprocal(1.0 + jnp.exp2(hp * -LOG2E), approx=True)
            h_scr[pl.ds(zs, T), c0:c1] = act.astype(bf16)

        bparts = {}

        def ffn2(c):
            bparts[c] = jnp.dot(h_scr[pl.ds(zl, T), :], w2_v[:, 128 * c:128 * c + 128], preferred_element_type=f32)

        if not first:
            ffn1(0, F)

        kr = lax.broadcasted_iota(jnp.int32, (64, 128), 0)
        ln = lax.broadcasted_iota(jnp.int32, (64, 128), 1)
        low = kr <= (ln & 63)
        ms = {}

        def nrows(u):
            return min(64 * (u + 1), WIN) if first else WIN

        def scores(n):
            u, j = divmod(n, NG)
            nr = nrows(u)
            qq = q_scr[pl.ds(zl + j * T + 64 * u, 64), :]
            qms = []
            for hh in range(4):
                b0 = (80 * j + 20 * hh) % 128
                e0 = b0 + 20
                mk = ((ln >= b0) & (ln < e0)) if e0 <= 128 else ((ln >= b0) | (ln < e0 - 128))
                qms.append(jnp.where(mk, qq, 0.0))
            qm = jnp.concatenate(qms, axis=0).astype(bf16)
            if first:
                kw = k_scr[j, 64 * (u + 1) - nr:64 * (u + 1), :]
            else:
                kw = k_scr[j, pl.ds(pl.multiple_of(ib * T + 64 * u - 256, 64), WIN), :]
            s = lax.dot_general(kw, qm, NT, preferred_element_type=f32)
            buf = sbuf[n % (LA + 1)]
            for p in range(2):
                sh = s[:, 128 * p:128 * p + 128]
                diag = sh[nr - 64:nr]
                if nr == WIN:
                    mg = jnp.where(low, diag, sh[0:64])
                    mid = sh[64:256]
                else:
                    mg = jnp.where(low, diag, NEG)
                    mid = sh[0:nr - 64] if nr > 64 else None
                buf[pl.ds(zs + 256 * p, 64), :] = mg
                mx = mg
                if mid is not None:
                    nm = mid.shape[0]
                    buf[pl.ds(zs + 256 * p + 64, nm), :] = mid
                    for b in range(nm // 64):
                        mx = jnp.maximum(mx, mid[64 * b:64 * b + 64])
                ms[(n, p)] = jnp.max(mx, axis=0, keepdims=True)

        def softmax_pv(n):
            u, j = divmod(n, NG)
            nr = nrows(u)
            buf = sbuf[n % (LA + 1)]
            kb = kb0 + u // 2
            nm = nr - 128 if nr == WIN else nr - 64
            z64 = jnp.zeros((64, 128), f32)
            for p in range(2):
                m = ms[(n, p)]
                e_mg = jnp.exp2(buf[pl.ds(zl + 256 * p, 64), :] - m)
                parts = []
                if nr == WIN:
                    parts.append(jnp.where(low, 0.0, e_mg))
                if nm:
                    parts.append(jnp.exp2(buf[pl.ds(zl + 256 * p + 64, nm), :] - m))
                parts.append(jnp.where(low, e_mg, 0.0) if nr == WIN else e_mg)
                if nr % 128:
                    if u % 2 == 0:
                        parts.append(z64)
                    else:
                        parts.insert(0, z64)
                pt = jnp.concatenate(parts, axis=0).astype(bf16)
                nt = pt.shape[0] // 128
                vw = jnp.concatenate([v_scr[2 * j + p, kb - (nt - 1) + i] for i in range(nt)], axis=1)
                oo = jnp.dot(vw, pt, preferred_element_type=f32)
                inv = 1.0 / (oo[40:48] if p == 0 else oo[0:8])
                body = oo[0:40] if p == 0 else oo[8:48]
                o_scr[u, pl.ds(zs + 80 * j + 40 * p, 40), :] = body * jnp.concatenate([inv] * 5, axis=0)

        ns = NU * NG
        for n in range(LA):
            scores(n)
        for n in range(ns):
            if n + LA < ns:
                scores(n + LA)
            elif first:
                fi = n - (ns - 2)
                if fi == 0:
                    wcp(W1).wait()
                if fi >= 0:
                    ffn1(fi * (F // 2), (fi + 1) * (F // 2))
            elif n == ns - 1:
                ffn2(0)
            softmax_pv(n)

        if first:
            wcp(WO).wait()
            wcp(W2).wait()
            wcp(GW).wait()
            ffn2(0)
        else:
            ffn2(1)
        dcol = lax.broadcasted_iota(jnp.int32, (64, D), 1)
        even = (((dcol * 205) >> 12) & 1) == 0
        obs = []
        for u in range(NU):
            z = o_scr[u, pl.ds(zl, D), :].T
            obs.append(jnp.where(even, z[0:64], z[64:128]))
        ob = jnp.concatenate(obs, axis=0).astype(bf16)
        aa = jnp.dot(ob, wo_v[...], preferred_element_type=f32)
        for c in range(1 if first else 2, 4):
            ffn2(c)
        gl = jnp.sum(x_ref[...].astype(f32) * gw_v[...].astype(f32).reshape(1, D), axis=1, keepdims=True)
        g = jax.nn.sigmoid(gl)
        for r in range(4):
            rs = slice(64 * r, 64 * r + 64)
            b4 = jnp.dot(h_scr[pl.ds(zl + 64 * r, 64), :], w2_v[:, 512:640], preferred_element_type=f32)
            for c in range(D // 128):
                cs = slice(128 * c, 128 * c + 128)
                bb = b4 if c == 4 else bparts[c][rs]
                out_v[slot, rs, cs] = (g[rs] * aa[rs, cs] + (1.0 - g[rs]) * bb).astype(bf16)
            ocp(0 if first else ib, slot, r).start()
        if not first:
            @pl.when(ib == S // T - 1)
            def _():
                for r in range(4):
                    ocp(ib - 1, 1 - slot, r).wait()
                for r in range(4):
                    ocp(ib, slot, r).wait()

    @pl.when(ib == 0)
    def _():
        step(True)

    @pl.when(ib > 0)
    def _():
        step(False)


@jax.jit
def pallas_gated_mix__sliding_block__dense_activation_silu__prompt_kernel(
        A_x, A_wqkv, A_wo, B_x, B_w1, B_w2, gate_w):
    del B_x
    any_spec = pl.BlockSpec(memory_space=pl.ANY)
    out = pl.pallas_call(
        _kernel,
        grid=(S // T,),
        in_specs=[any_spec] * 6,
        out_specs=any_spec,
        out_shape=jax.ShapeDtypeStruct((S, D), bf16),
        scratch_shapes=[
            pltpu.VMEM((2, T, D), bf16),
            pltpu.VMEM((2, T, D), bf16),
            pltpu.VMEM((D,), bf16),
            pltpu.VMEM((D, 3 * D), bf16),
            pltpu.VMEM((D, D), bf16),
            pltpu.VMEM((D, F), bf16),
            pltpu.VMEM((F, D), bf16),
            pltpu.VMEM((NG, S, 128), bf16),
            pltpu.VMEM((H // 2, S // 128, 48, 128), bf16),
            pltpu.VMEM((NG * T, 128), f32),
            pltpu.VMEM((T, F), bf16),
            pltpu.VMEM((NU, D, 128), f32),
            pltpu.SemaphoreType.DMA((NP + 4,)),
            pltpu.SemaphoreType.DMA((2,)),
            pltpu.SemaphoreType.DMA((8,)),
        ] + [pltpu.VMEM((512, 128), f32)] * (LA + 1),
        compiler_params=pltpu.CompilerParams(
            dimension_semantics=("arbitrary",),
            vmem_limit_bytes=100 * 1024 * 1024),
    )(A_x.reshape(S, D), gate_w, A_wqkv, A_wo, B_w1, B_w2)
    return out.reshape(1, S, D)
```
